```python
import jax
import jax.numpy as jnp

def _softmax(x, axis=-1):
    return jax.nn.softmax(x, axis=axis)
def _gelu(x):
    return jax.nn.gelu(x, approximate=True)
def _silu(x):
    return jax.nn.silu(x)
def _sigmoid(x):
    return jax.nn.sigmoid(x)
def _layernorm(x, axis=-1, eps=1e-5):
    m = jnp.mean(x, axis=axis, keepdims=True)
    v = jnp.var(x, axis=axis, keepdims=True)
    return (x - m) / jnp.sqrt(v + eps)
def _scatter_add(tgt, idx, src, axis=0):
    return tgt.at[idx].add(src)
def _segment_sum(src, seg, n):
    return jax.ops.segment_sum(src, seg, n)
class _Rng:
    def __init__(self, key):
        self._k = key
    def _next(self):
        self._k, sub = jax.random.split(self._k)
        return sub
    def normal(self, shape):
        return jax.random.normal(self._next(), shape, dtype=jnp.bfloat16)
    def randint(self, lo, hi, shape):
        return jax.random.randint(self._next(), shape, lo, hi, dtype=jnp.int32)
    def uniform(self, shape, lo=0.0, hi=1.0):
        return jax.random.uniform(self._next(), shape, jnp.bfloat16, lo, hi)
    def permutation(self, n):
        return jax.random.permutation(self._next(), n)


kernel_name = 'sequential_preLN__grouped_kv_mqa__glu_gated_swiglu__prompt'

def _fwd_setup_inputs():
    _rng = _Rng(jax.random.key(int.from_bytes(__import__("os").urandom(4), "little")))
    _w = (lambda a: (lambda t: t.astype(jnp.bfloat16) if jnp.issubdtype(t.dtype, jnp.floating) else t)(jnp.asarray(a)))
    def _A_setup():
        B, S, D, H = 1, 2048, 512, 32
        Dh = D // H
        return {
            "x": _w((lambda *s: _rng.normal(s) * 0.05)(B, S, D)),
            "wq": _w((lambda *s: _rng.normal(s) * 0.05)(D, H * Dh)),
            "wk": _w((lambda *s: _rng.normal(s) * 0.05)(D, Dh)),
            "wv": _w((lambda *s: _rng.normal(s) * 0.05)(D, Dh)),
            "wo": _w((lambda *s: _rng.normal(s) * 0.05)(H * Dh, D)),
        }
    _A_in = _A_setup()

    def _B_setup():
        B, S, D, F = 1, 2048, 512, 1376
        return {
            "x": _w((lambda *s: _rng.normal(s) * 0.05)(B, S, D)),
            "w1": _w((lambda *s: _rng.normal(s) * 0.05)(D, F) * (2.0 / D) ** 0.5),
            "w3": _w((lambda *s: _rng.normal(s) * 0.05)(D, F) * (2.0 / D) ** 0.5),
            "w2": _w((lambda *s: _rng.normal(s) * 0.05)(F, D) * (2.0 / F) ** 0.5),
        }
    _B_in = _B_setup()

    return {
        "A_x": _A_in["x"],
        "A_wq": _A_in["wq"],
        "A_wk": _A_in["wk"],
        "A_wv": _A_in["wv"],
        "A_wo": _A_in["wo"],
        "B_x": _B_in["x"],
        "B_w1": _B_in["w1"],
        "B_w3": _B_in["w3"],
        "B_w2": _B_in["w2"],
    }

def _fwd_reference(A_x, A_wq, A_wk, A_wv, A_wo, B_x, B_w1, B_w3, B_w2):
    def _A_ref(x, wq, wk, wv, wo):
        B, S, D = x.shape
        H = 32
        Dh = D // H
        q = (lambda x, *d: x.transpose(*d))((x @ wq).reshape(B, S, H, Dh), 0, 2, 1, 3)
        k = x @ wk
        v = x @ wv
        scores = jnp.einsum("bhqd,bkd->bhqk", q, k) * (Dh ** -0.5)
        p = _softmax(scores, axis=-1)
        o = jnp.einsum("bhqk,bkd->bhqd", p, v)
        return (lambda x, *d: x.transpose(*d))(o, 0, 2, 1, 3).reshape(B, S, H * Dh) @ wo

    def _B_ref(x, w1, w3, w2):
        gate = jnp.einsum("bsd,df->bsf", x, w1)
        up = jnp.einsum("bsd,df->bsf", x, w3)
        h = _silu(gate) * up
        out = jnp.einsum("bsf,fd->bsd", h, w2)
        return out

    x = A_x
    h = x + _A_ref(_layernorm(x, axis=-1), A_wq, A_wk, A_wv, A_wo)
    h2 = h + _B_ref(_layernorm(h, axis=-1), B_w1, B_w3, B_w2)
    return h2


def setup_inputs():
    _inp = _fwd_setup_inputs()
    _gk = jax.random.fold_in(jax.random.key(int.from_bytes(__import__("os").urandom(4), "little")), 2**31 - 1)
    _shapes = [[1, 2048, 512]]
    _dtypes = ['bfloat16']
    _gks = jax.random.split(_gk, len(_shapes))
    _gs = [jax.random.normal(k, s, dtype=jnp.dtype(d)) * 0.05 for k, s, d in zip(_gks, _shapes, _dtypes)]
    _inp["grad_out"] = _gs[0]
    return _inp

def reference(A_x, A_wq, A_wk, A_wv, A_wo, B_w1, B_w3, B_w2, B_x, grad_out):
    _const = dict(B_x=B_x)
    def _f(*_d):
        return _fwd_reference(**{'A_x': _d[0], 'A_wq': _d[1], 'A_wk': _d[2], 'A_wv': _d[3], 'A_wo': _d[4], 'B_w1': _d[5], 'B_w3': _d[6], 'B_w2': _d[7], **_const})
    _out, _vjp = jax.vjp(_f, A_x, A_wq, A_wk, A_wv, A_wo, B_w1, B_w3, B_w2)
    _grads = _vjp(grad_out)
    _out0 = jnp.asarray(_out)
    return (_out0, *[jnp.asarray(_g) for _g in _grads])
```

```python
import math

import jax
import jax.numpy as jnp
from jax import lax
import jax.experimental.pallas as pl
import jax.experimental.pallas.tpu as pltpu

f32 = jnp.float32
bf16 = jnp.bfloat16

S = 2048
D = 512
H = 32
DH = 16
F = 1376
EPS = 1e-5

TQ = 512
NQ = S // TQ
BK = 128
NKC = S // BK
FC = 256

LOG2E = math.log2(math.e)
LN2 = math.log(2.0)
SCALE = DH ** -0.5
QSCALE = SCALE * LOG2E
SAFE_BOUND = 40.0

NT = (((1,), (1,)), ((), ()))


def _dot(a, b):
    return jnp.dot(a, b, preferred_element_type=f32)


def _dot_nt(a, b):
    return lax.dot_general(a, b, NT, preferred_element_type=f32)


def _ln_fwd_fm(xt):
    mean = jnp.sum(xt, axis=0, keepdims=True) * (1.0 / D)
    xc = xt - mean
    var = jnp.sum(xc * xc, axis=0, keepdims=True) * (1.0 / D)
    rstd = lax.rsqrt(var + EPS)
    return xc * rstd, rstd


def _ln_bwd_fm(dy, xn, rstd):
    m1 = jnp.sum(dy, axis=0, keepdims=True) * (1.0 / D)
    m2 = jnp.sum(dy * xn, axis=0, keepdims=True) * (1.0 / D)
    return rstd * (dy - m1 - xn * m2)


def _chunks(n, c):
    return [(lo, min(c, n - lo)) for lo in range(0, n, c)]


def _kernel(
    x_hbm, wq_hbm, wkT_ref, wvT_ref, wo_hbm, w1T_hbm, w3T_hbm, w2_hbm, g_hbm,
    h2_hbm, dx_hbm, dwq_hbm, dwkT_ref, dwvT_ref, dwo_hbm, dw1T_hbm, dw3T_hbm, dw2_hbm,
    xT, xnT, rstd1,
    wq_s, wqT, wo_s, woT, w1_s, w3_s, w2_s, w1T, w3T, w2T,
    kaug, vaug, kT, vT,
    qT, maug, doT, daug, oT32, oT, linv,
    pE, pO, dsE, dsO,
    dqT, dhT, dkT, dvT,
    dw1a, dw3a, dw2a, dwoa,
    aT, dgT, duT,
    hT, hnT, gT, outa, dhna,
    gbuf, obuf, xbuf,
    sems, osem,
):
    def x_copy(t):
        return pltpu.make_async_copy(x_hbm.at[pl.ds(t * TQ, TQ), :], xbuf.at[pl.ds(t * TQ, TQ), :], sems.at[t])

    def g_copy(j):
        return pltpu.make_async_copy(g_hbm.at[pl.ds(pl.multiple_of(j * TQ, TQ), TQ), :], gbuf, sems.at[4])

    w_copies = [
        pltpu.make_async_copy(wq_hbm, wq_s, sems.at[5]),
        pltpu.make_async_copy(wo_hbm, wo_s, sems.at[6]),
        pltpu.make_async_copy(w2_hbm, w2_s, sems.at[7]),
        pltpu.make_async_copy(w1T_hbm, w1T, sems.at[8]),
        pltpu.make_async_copy(w3T_hbm, w3T, sems.at[9]),
    ]
    for t in range(NQ):
        x_copy(t).start()
    w_copies[0].start()
    g_copy(0).start()
    for c in w_copies[1:]:
        c.start()

    dw1a[...] = jnp.zeros_like(dw1a)
    dw3a[...] = jnp.zeros_like(dw3a)
    dw2a[...] = jnp.zeros_like(dw2a)
    dwoa[...] = jnp.zeros_like(dwoa)
    dkT[...] = jnp.zeros_like(dkT)
    dvT[...] = jnp.zeros_like(dvT)

    wkvT = jnp.concatenate([wkT_ref[...], wvT_ref[...]], axis=0)
    row16 = lax.broadcasted_iota(jnp.int32, (DH, TQ), 0)
    kaug_tail = jnp.where(row16 < 2, -1.0, 0.0).astype(bf16)
    kmax2 = jnp.zeros((1, TQ), f32)
    for t in range(NQ):
        ts = slice(t * TQ, (t + 1) * TQ)
        x_copy(t).wait()
        xt_b = xbuf[ts, :].T
        xT[:, ts] = xt_b
        xn, r = _ln_fwd_fm(xt_b.astype(f32))
        xn_b = xn.astype(bf16)
        xnT[:, ts] = xn_b
        rstd1[:, ts] = jnp.broadcast_to(r, (8, TQ))
        kv = _dot(wkvT, xn_b).astype(bf16)
        kT[:, ts] = kv[:DH]
        vT[:, ts] = kv[DH:]
        kf = kv[:DH].astype(f32)
        kmax2 = jnp.maximum(kmax2, jnp.sum(kf * kf, axis=0, keepdims=True))
        kaug[ts, :] = jnp.concatenate([kv[:DH], kaug_tail], axis=0).T
        vaug[ts, :] = jnp.concatenate([kv[DH:], kaug_tail], axis=0).T
    kmax = jnp.sqrt(jnp.max(kmax2, axis=1, keepdims=True)) * 1.01

    w_copies[0].wait()
    wqT[...] = wq_s[...].T
    w_copies[1].wait()
    woT[...] = wo_s[...].T
    w_copies[2].wait()
    w2T[...] = w2_s[...].T
    w_copies[3].wait()
    w1_s[...] = w1T[...].T
    w_copies[4].wait()
    w3_s[...] = w3T[...].T

    def head_rows(h):
        return pl.ds(pl.multiple_of(h * DH, DH), DH)

    def aug_tile(vals_ref, aug_ref, h):
        a = aug_ref[pl.ds(h, 1), :]
        hi = a.astype(bf16).astype(f32)
        lo = a - hi
        tail = jnp.where(row16 == 0, hi, jnp.where(row16 == 1, lo, 0.0)).astype(bf16)
        return jnp.concatenate([vals_ref[head_rows(h), :], tail], axis=0)

    def fwd_step(h_prod, p_prod, i_prod, h_cons, p_cons, i_cons, l_prev):
        if h_prod is not None:
            w = aug_tile(qT, maug, h_prod)
            lacc = jnp.zeros((8, TQ), f32)
        if h_cons is not None:
            acc = jnp.zeros((DH, TQ), f32)
        for kc in range(NKC):
            ks = slice(kc * BK, (kc + 1) * BK)
            if h_prod is not None:
                p = jnp.exp2(_dot(kaug[ks, :], w))
                p_prod[i_prod, ks, :] = p.astype(bf16)
                lacc = lacc + p.reshape(BK // 8, 8, TQ).sum(0)
            if h_cons is not None:
                acc = acc + _dot(vT[:, ks], p_cons[i_cons, ks, :])
        if h_cons is not None:
            o = acc * l_prev
            oT32[head_rows(h_cons), :] = o
            oT[head_rows(h_cons), :] = o.astype(bf16)
            linv[pl.ds(h_cons, 1), :] = l_prev
        if h_prod is not None:
            return 1.0 / jnp.sum(lacc, axis=0, keepdims=True)
        return None

    def bwd_step(h_prod, p_prod, i_prod, ds_prod, h_cons, p_cons, i_cons, ds_cons, q0):
        if h_prod is not None:
            w = aug_tile(doT, daug, h_prod)
        if h_cons is not None:
            dq = jnp.zeros((DH, TQ), f32)
            do_c = doT[head_rows(h_cons), :]
            q_c = qT[head_rows(h_cons), :]
        for kc in range(NKC):
            ks = slice(kc * BK, (kc + 1) * BK)
            if h_prod is not None:
                dp = _dot(vaug[ks, :], w)
                ds_prod[ks, :] = (p_prod[i_prod, ks, :].astype(f32) * dp).astype(bf16)
            if h_cons is not None:
                dvT[:, ks] += _dot_nt(do_c, p_cons[i_cons, ks, :])
                dkT[:, ks] += _dot_nt(q_c, ds_cons[ks, :])
                dq = dq + _dot(kT[:, ks], ds_cons[ks, :])
        if h_cons is not None:
            dqT[head_rows(h_cons), pl.ds(q0, TQ)] = (dq * SCALE).astype(bf16)

    def tile_body(j, _):
        q0 = pl.multiple_of(j * TQ, TQ)
        qs = pl.ds(q0, TQ)

        xn_b = xnT[:, qs]
        q_b = (_dot(wqT[...], xn_b) * QSCALE).astype(bf16)
        qT[...] = q_b
        qf = q_b.astype(f32)
        qn2 = jnp.sum((qf * qf).reshape(H, DH, TQ), axis=1)
        bound = jnp.sqrt(qn2) * kmax
        maug[...] = bound

        @pl.when(jnp.max(bound) > SAFE_BOUND)
        def _():
            def true_max(h, _):
                w = qT[head_rows(h), :]
                m = jnp.full((8, TQ), -jnp.inf, f32)
                for kc in range(NKC):
                    s = _dot(kaug[kc * BK:(kc + 1) * BK, 0:DH], w)
                    m = jnp.maximum(m, s.reshape(BK // 8, 8, TQ).max(0))
                maug[pl.ds(h, 1), :] = jnp.max(m, axis=0, keepdims=True)
                return 0
            lax.fori_loop(0, H, true_max, 0)

        l0 = fwd_step(0, pE, 0, None, None, None, None)

        def fwd_loop(i, l_prev):
            l1 = fwd_step(2 * i + 1, pO, i, 2 * i, pE, i, l_prev)
            return fwd_step(2 * i + 2, pE, i + 1, 2 * i + 1, pO, i, l1)

        l_last = lax.fori_loop(0, H // 2 - 1, fwd_loop, l0)
        l_last = fwd_step(H - 1, pO, H // 2 - 1, H - 2, pE, H // 2 - 1, l_last)
        fwd_step(None, None, None, H - 1, pO, H // 2 - 1, l_last)

        h_f = xT[:, qs].astype(f32) + _dot(woT[...], oT[...])
        hT[...] = h_f
        g_copy(j).wait()
        g_b = gbuf[...].T
        gT[...] = g_b

        @pl.when(j + 1 < NQ)
        def _():
            g_copy(j + 1).start()

        hn, r2 = _ln_fwd_fm(h_f)
        hn_b = hn.astype(bf16)
        hnT[...] = hn_b

        fch = _chunks(F, FC)

        def produce(lo, n):
            fs = slice(lo, lo + n)
            da = _dot(w2_s[fs, :], gT[...])
            gate = _dot(w1T[fs, :], hnT[...])
            up = _dot(w3T[fs, :], hnT[...])
            sig = jax.nn.sigmoid(gate)
            silu = gate * sig
            aT[fs, :] = (silu * up).astype(bf16)
            duT[fs, :] = (da * silu).astype(bf16)
            dgT[fs, :] = (da * up * (sig + silu * (1.0 - sig))).astype(bf16)

        def consume(lo, n, first):
            fs = slice(lo, lo + n)
            o_c = _dot(w2T[:, fs], aT[fs, :])
            d_c = _dot(w1_s[:, fs], dgT[fs, :]) + _dot(w3_s[:, fs], duT[fs, :])
            if first:
                outa[...] = o_c
                dhna[...] = d_c
            else:
                outa[...] += o_c
                dhna[...] += d_c
            dw2a[fs, :] += _dot_nt(aT[fs, :], gT[...])
            dw1a[fs, :] += _dot_nt(dgT[fs, :], hnT[...])
            dw3a[fs, :] += _dot_nt(duT[fs, :], hnT[...])

        for c, (lo, n) in enumerate(fch):
            produce(lo, n)
            if c > 0:
                consume(*fch[c - 1], c == 1)
        consume(*fch[-1], False)

        @pl.when(j > 0)
        def _():
            pltpu.make_async_copy(obuf, h2_hbm.at[qs, :], osem.at[0]).wait()

        obuf[...] = (hT[...] + outa[...]).astype(bf16).T
        pltpu.make_async_copy(obuf, h2_hbm.at[qs, :], osem.at[0]).start()

        dh = gT[...].astype(f32) + _ln_bwd_fm(dhna[...], hnT[...].astype(f32), r2)
        dh_b = dh.astype(bf16)
        dhT[:, qs] = dh_b
        do = _dot(wo_s[...], dh_b)
        dwoa[...] += _dot_nt(oT[...], dh_b)
        li = linv[...]
        do_b = (do.reshape(H, DH, TQ) * li[:, None, :]).astype(bf16)
        doT[...] = do_b.reshape(H * DH, TQ)
        daug[...] = jnp.sum(do_b.astype(f32) * oT32[...].reshape(H, DH, TQ), axis=1)

        @pl.when(j == NQ - 1)
        def _():
            w1T[...] = dw1a[...].astype(bf16)
            w3T[...] = dw3a[...].astype(bf16)
            w2_s[...] = dw2a[...].astype(bf16)
            wo_s[...] = dwoa[...].astype(bf16)
            pltpu.make_async_copy(w1T, dw1T_hbm, sems.at[8]).start()
            pltpu.make_async_copy(w3T, dw3T_hbm, sems.at[9]).start()
            pltpu.make_async_copy(w2_s, dw2_hbm, sems.at[7]).start()
            pltpu.make_async_copy(wo_s, dwo_hbm, sems.at[6]).start()

        bwd_step(0, pE, 0, dsE, None, None, None, None, q0)

        def bwd_loop(i, _):
            bwd_step(2 * i + 1, pO, i, dsO, 2 * i, pE, i, dsE, q0)
            bwd_step(2 * i + 2, pE, i + 1, dsE, 2 * i + 1, pO, i, dsO, q0)
            return 0

        lax.fori_loop(0, H // 2 - 1, bwd_loop, 0)
        bwd_step(H - 1, pO, H // 2 - 1, dsO, H - 2, pE, H // 2 - 1, dsE, q0)
        bwd_step(None, None, None, None, H - 1, pO, H // 2 - 1, dsO, q0)
        return 0

    lax.fori_loop(0, NQ, tile_body, 0)

    dk_b = (dkT[...] * LN2).astype(bf16)
    dv_b = dvT[...].astype(bf16)
    dkv_b = jnp.concatenate([dk_b, dv_b], axis=0)
    dwkvT = _dot_nt(dkv_b, xnT[...]).astype(bf16)
    dwkT_ref[...] = dwkvT[:DH]
    dwvT_ref[...] = dwkvT[DH:]
    wkv = wkvT.T
    wqT[...] = _dot_nt(xnT[...], dqT[...]).astype(bf16)
    dwq_copy = pltpu.make_async_copy(wqT, dwq_hbm, sems.at[5])
    dwq_copy.start()

    def dx_copy(t):
        return pltpu.make_async_copy(xbuf.at[pl.ds(t * TQ, TQ), :], dx_hbm.at[pl.ds(t * TQ, TQ), :], sems.at[t])

    for t in range(NQ):
        ts = slice(t * TQ, (t + 1) * TQ)
        dxn = _dot(wq_s[...], dqT[:, ts]) + _dot(wkv, dkv_b[:, ts])
        dx = dhT[:, ts].astype(f32) + _ln_bwd_fm(dxn, xnT[:, ts].astype(f32), rstd1[0:1, ts])
        xbuf[ts, :] = dx.astype(bf16).T
        dx_copy(t).start()

    pltpu.make_async_copy(obuf, h2_hbm.at[pl.ds(0, TQ), :], osem.at[0]).wait()
    pltpu.make_async_copy(w1T, dw1T_hbm, sems.at[8]).wait()
    pltpu.make_async_copy(w3T, dw3T_hbm, sems.at[9]).wait()
    pltpu.make_async_copy(w2_s, dw2_hbm, sems.at[7]).wait()
    pltpu.make_async_copy(wo_s, dwo_hbm, sems.at[6]).wait()
    dwq_copy.wait()
    for t in range(NQ):
        dx_copy(t).wait()


@jax.jit
def pallas_sequential_preLN__grouped_kv_mqa__glu_gated_swiglu__prompt_kernel(
    A_x: jax.Array,
    A_wq: jax.Array,
    A_wk: jax.Array,
    A_wv: jax.Array,
    A_wo: jax.Array,
    B_x: jax.Array,
    B_w1: jax.Array,
    B_w3: jax.Array,
    B_w2: jax.Array,
    grad_out: jax.Array,
):
    del B_x
    V = pltpu.VMEM
    any_spec = pl.BlockSpec(memory_space=pl.ANY)
    vmem_spec = pl.BlockSpec(memory_space=pltpu.VMEM)
    scratch = [
        V((D, S), bf16), V((D, S), bf16), V((8, S), f32),
        V((D, D), bf16), V((D, D), bf16), V((D, D), bf16), V((D, D), bf16),
        V((D, F), bf16), V((D, F), bf16), V((F, D), bf16),
        V((F, D), bf16), V((F, D), bf16), V((D, F), bf16),
        V((S, 2 * DH), bf16), V((S, 2 * DH), bf16), V((DH, S), bf16), V((DH, S), bf16),
        V((D, TQ), bf16), V((H, TQ), f32), V((D, TQ), bf16), V((H, TQ), f32),
        V((D, TQ), f32), V((D, TQ), bf16), V((H, TQ), f32),
        V((H // 2, S, TQ), bf16), V((H // 2, S, TQ), bf16),
        V((S, TQ), bf16), V((S, TQ), bf16),
        V((D, S), bf16), V((D, S), bf16), V((DH, S), f32), V((DH, S), f32),
        V((F, D), f32), V((F, D), f32), V((F, D), f32), V((D, D), f32),
        V((F, TQ), bf16), V((F, TQ), bf16), V((F, TQ), bf16),
        V((D, TQ), f32), V((D, TQ), bf16), V((D, TQ), bf16), V((D, TQ), f32), V((D, TQ), f32),
        V((TQ, D), bf16), V((TQ, D), bf16), V((S, D), bf16),
        pltpu.SemaphoreType.DMA((10,)), pltpu.SemaphoreType.DMA((1,)),
    ]
    sds = jax.ShapeDtypeStruct
    out_shape = (
        sds((S, D), bf16), sds((S, D), bf16),
        sds((D, H * DH), bf16), sds((DH, D), bf16), sds((DH, D), bf16), sds((H * DH, D), bf16),
        sds((F, D), bf16), sds((F, D), bf16), sds((F, D), bf16),
    )
    outs = pl.pallas_call(
        _kernel,
        out_shape=out_shape,
        in_specs=[any_spec, any_spec, vmem_spec, vmem_spec, any_spec, any_spec, any_spec, any_spec, any_spec],
        out_specs=(any_spec, any_spec, any_spec, vmem_spec, vmem_spec, any_spec, any_spec, any_spec, any_spec),
        scratch_shapes=scratch,
        compiler_params=pltpu.CompilerParams(vmem_limit_bytes=127 * 1024 * 1024),
        name="preln_mqa_swiglu_fwdbwd",
    )(A_x.reshape(S, D), A_wq, A_wk.T, A_wv.T, A_wo, B_w1.T, B_w3.T, B_w2, grad_out.reshape(S, D))
    h2, dx, dwq, dwkT, dwvT, dwo, dw1T, dw3T, dw2 = outs
    return (h2.reshape(1, S, D), dx.reshape(1, S, D), dwq, dwkT.T, dwvT.T, dwo, dw1T.T, dw3T.T, dw2)
```

```python
import contextlib
import math

import jax
import jax.numpy as jnp
from jax import lax
import jax.experimental.pallas as pl
import jax.experimental.pallas.tpu as pltpu

f32 = jnp.float32
bf16 = jnp.bfloat16
u32 = jnp.uint32

S = 2048
D = 512
H = 32
DH = 16
F = 1376
EPS = 1e-5

TQ = 512
NQ = S // TQ
BK = 128
NKC = S // BK
FC = 256
TX = 512
FWD_UNROLL = 3
BWD_UNROLL = 3

LOG2E = math.log2(math.e)
LN2 = math.log(2.0)
SCALE = DH ** -0.5
QSCALE = SCALE * LOG2E
SAFE_BOUND = 40.0

NT = (((1,), (1,)), ((), ()))
PROFILE_SCOPES = False


def _scope(name):
    return jax.named_scope(name) if PROFILE_SCOPES else contextlib.nullcontext()


def _dot(a, b):
    return jnp.dot(a, b, preferred_element_type=f32)


def _dot_nt(a, b):
    return lax.dot_general(a, b, NT, preferred_element_type=f32)


def _ln_fwd_fm(xt):
    mean = jnp.sum(xt, axis=0, keepdims=True) * (1.0 / D)
    xc = xt - mean
    var = jnp.sum(xc * xc, axis=0, keepdims=True) * (1.0 / D)
    rstd = lax.rsqrt(var + EPS)
    return xc * rstd, rstd


def _ln_bwd_fm(dy, xn, rstd):
    m1 = jnp.sum(dy, axis=0, keepdims=True) * (1.0 / D)
    m2 = jnp.sum(dy * xn, axis=0, keepdims=True) * (1.0 / D)
    return rstd * (dy - m1 - xn * m2)


def _loop(n, body, carry, unroll):
    assert n % unroll == 0
    if unroll == n:
        for i in range(n):
            carry = body(i, carry)
        return carry

    def outer(i, c):
        for u in range(unroll):
            c = body(i * unroll + u, c)
        return c
    return lax.fori_loop(0, n // unroll, outer, carry)


def _pack(x):
    return pltpu.bitcast(x.astype(bf16), jnp.uint32)


def _unpack(x):
    return pltpu.bitcast(x, bf16)


def _chunks(n, c):
    return [(lo, min(c, n - lo)) for lo in range(0, n, c)]


def _kernel(
    x_hbm, wq_hbm, wkT_hbm, wvT_hbm, wo_hbm, w1T_hbm, w3T_hbm, w2_hbm, g_hbm,
    h2_hbm, dx_hbm, dwq_hbm, dwkT_hbm, dwvT_hbm, dwo_hbm, dw1T_hbm, dw3T_hbm, dw2_hbm,
    xT, xnT, rstd1,
    wq_s, wqT, wo_s, woT, w1_s, w3_s, w2_s, w1T, w3T, w2T,
    kaug, vaug, kT, vT,
    qT, maug, doT, daug, oT32, oT, linv,
    pE, pO, dsE, dsO,
    dqT, dhT, dkT, dvT, dkvT,
    dw1a, dw3a, dw2a, dwoa, dwqa,
    aT, dgT, duT,
    hnT, gT, outa, dhna,
    gbuf, obuf, xbuf, wkvT_s, dwkvT_s,
    sems, osem, xsem,
):
    def x_copy(t):
        return pltpu.make_async_copy(x_hbm.at[pl.ds(t * TQ, TQ), :], xbuf.at[pl.ds(t * TQ, TQ), :], sems.at[t])

    def g_copy(j):
        return pltpu.make_async_copy(g_hbm.at[pl.ds(j * TQ, TQ), :], gbuf, sems.at[4])

    w_copies = [
        pltpu.make_async_copy(wq_hbm, wq_s, sems.at[5]),
        pltpu.make_async_copy(wo_hbm, wo_s, sems.at[6]),
        pltpu.make_async_copy(w2_hbm, w2_s, sems.at[7]),
        pltpu.make_async_copy(w1T_hbm, w1T, sems.at[8]),
        pltpu.make_async_copy(w3T_hbm, w3T, sems.at[9]),
    ]
    kv_copies = [
        pltpu.make_async_copy(wkT_hbm, wkvT_s.at[pl.ds(0, DH), :], sems.at[10]),
        pltpu.make_async_copy(wvT_hbm, wkvT_s.at[pl.ds(DH, DH), :], sems.at[11]),
    ]
    x_copy(0).start()
    for c in kv_copies:
        c.start()
    for t in range(1, NQ):
        x_copy(t).start()
    w_copies[0].start()
    g_copy(0).start()
    for c in w_copies[1:]:
        c.start()

    with _scope("zero"):
        dkT[...] = jnp.zeros_like(dkT)
        dvT[...] = jnp.zeros_like(dvT)

    with _scope("ln1kv"):
        for c in kv_copies:
            c.wait()
        wkvT = wkvT_s[...]
        row16 = lax.broadcasted_iota(jnp.int32, (DH, TQ), 0)
        kaug_tail = jnp.where(row16 < 2, -1.0, 0.0).astype(bf16)
        kmax2 = jnp.zeros((1, TQ), f32)
        for t in range(NQ):
            ts = slice(t * TQ, (t + 1) * TQ)
            x_copy(t).wait()
            xt_b = xbuf[ts, :].T
            xT[:, ts] = xt_b
            xn, r = _ln_fwd_fm(xt_b.astype(f32))
            xn_b = xn.astype(bf16)
            xnT[:, ts] = xn_b
            rstd1[:, ts] = jnp.broadcast_to(r, (8, TQ))
            kv = _dot(wkvT, xn_b).astype(bf16)
            kT[:, ts] = kv[:DH]
            vT[:, ts] = kv[DH:]
            kf = kv[:DH].astype(f32)
            kmax2 = jnp.maximum(kmax2, jnp.sum(kf * kf, axis=0, keepdims=True))
            kaug[ts, :] = jnp.concatenate([kv[:DH], kaug_tail], axis=0).T
            vaug[ts, :] = jnp.concatenate([kv[DH:], kaug_tail], axis=0).T
        kmax = jnp.sqrt(jnp.max(kmax2, axis=1, keepdims=True)) * 1.01

    w_copies[0].wait()
    wqT[...] = wq_s[...].T

    def head_rows(h):
        return pl.ds(pl.multiple_of(h * DH, DH), DH)

    def aug_tile(vals_ref, aug_ref, h):
        a = aug_ref[pl.ds(h, 1), :]
        hi = a.astype(bf16).astype(f32)
        lo = a - hi
        tail = jnp.where(row16 == 0, hi, jnp.where(row16 == 1, lo, 0.0)).astype(bf16)
        return jnp.concatenate([vals_ref[head_rows(h), :], tail], axis=0)

    def attn_step(fprod=None, fcons=None, bprod=None, bcons=None, filler=None):
        if fprod:
            wf = aug_tile(qT, maug, fprod[0])
            lacc = jnp.zeros((8, TQ), f32)
        if fcons:
            acc = jnp.zeros((DH, TQ), f32)
        if bprod:
            wb = aug_tile(doT, daug, bprod[0])
        if bcons:
            dq = jnp.zeros((DH, TQ), f32)
            do_c = doT[head_rows(bcons[0]), :]
            q_c = qT[head_rows(bcons[0]), :] if bcons[5] is None else bcons[5]
        for kc in range(NKC):
            ks = slice(kc * BK, (kc + 1) * BK)
            ks2 = slice(kc * BK // 2, (kc + 1) * BK // 2)
            if fprod:
                p = jnp.exp2(_dot(kaug[ks, :], wf))
                fprod[1][fprod[2], ks2, :] = _pack(p)
                lacc = lacc + p.reshape(BK // 8, 8, TQ).sum(0)
            if bprod:
                dp = _dot(vaug[ks, :], wb)
                bprod[3][ks2, :] = _pack(_unpack(bprod[1][bprod[2], ks2, :]).astype(f32) * dp)
            if fcons:
                acc = acc + _dot(vT[:, ks], _unpack(fcons[1][fcons[2], ks2, :]))
            if bcons:
                ds_c = _unpack(bcons[3][ks2, :])
                dvT[:, ks] += _dot_nt(do_c, _unpack(bcons[1][bcons[2], ks2, :]))
                dkT[:, ks] += _dot_nt(q_c, ds_c)
                dq = dq + _dot(kT[:, ks], ds_c)
            if filler:
                filler(kc)
        if bcons:
            dqT[head_rows(bcons[0]), pl.ds(bcons[4], TQ)] = (dq * SCALE).astype(bf16)
        if fcons:
            h, l = fcons[0], fcons[3]
            o = acc * l
            oT32[head_rows(h), :] = o
            oT[head_rows(h), :] = o.astype(bf16)
            linv[pl.ds(h, 1), :] = l
        if fprod:
            return 1.0 / jnp.sum(lacc, axis=0, keepdims=True)
        return None

    def q_proj(j):
        with _scope("qproj"):
            q_b = (_dot(wqT[...], xnT[:, j * TQ:(j + 1) * TQ]) * QSCALE).astype(bf16)
            qT[...] = q_b
            qf = q_b.astype(f32)
            qn2 = jnp.sum((qf * qf).reshape(H, DH, TQ), axis=1)
            bound = jnp.sqrt(qn2) * kmax
            maug[...] = bound

            @pl.when(jnp.max(bound) > SAFE_BOUND)
            def _():
                def true_max(h, _):
                    w = qT[head_rows(h), :]
                    m = jnp.full((8, TQ), -jnp.inf, f32)
                    for kc in range(NKC):
                        s = _dot(kaug[kc * BK:(kc + 1) * BK, 0:DH], w)
                        m = jnp.maximum(m, s.reshape(BK // 8, 8, TQ).max(0))
                    maug[pl.ds(h, 1), :] = jnp.max(m, axis=0, keepdims=True)
                    return 0
                lax.fori_loop(0, H, true_max, 0)

    last = H // 2 - 1

    def tile_body(j, l0):
        q0 = j * TQ
        qs = pl.ds(q0, TQ)

        with _scope("attn_fwd"):
            def fwd_loop(i, l_prev):
                l1 = attn_step(fprod=(2 * i + 1, pO, i), fcons=(2 * i, pE, i, l_prev))
                return attn_step(fprod=(2 * i + 2, pE, i + 1), fcons=(2 * i + 1, pO, i, l1))

            l_last = _loop(last, fwd_loop, l0, FWD_UNROLL)
            g_copy(j).wait()
            gT[...] = gbuf[...].T
            if j + 1 < NQ:
                g_copy(j + 1).start()
            l_last = attn_step(fprod=(H - 1, pO, last), fcons=(H - 2, pE, last, l_last))
            da0 = _dot(w2_s[0:FC, :], gT[...]) if j > 0 else None
            attn_step(fcons=(H - 1, pO, last, l_last))

        if j == 0:
            w_copies[2].wait()
            da0 = _dot(w2_s[0:FC, :], gT[...])
            w2T[...] = w2_s[...].T
            w_copies[1].wait()
            woT[...] = wo_s[...].T
            w_copies[3].wait()
            w1_s[...] = w1T[...].T
            w_copies[4].wait()
            w3_s[...] = w3T[...].T

        with _scope("dense"):
            if j > 0:
                pltpu.make_async_copy(obuf, h2_hbm.at[qs, :], osem.at[0]).wait()

            h_f = xT[:, qs].astype(f32) + _dot(woT[...], oT[...])
            outa[...] = h_f
            hn, r2 = _ln_fwd_fm(h_f)
            hnT[...] = hn.astype(bf16)

            fch = _chunks(F, FC)

            def produce(lo, n):
                fs = slice(lo, lo + n)
                da = da0 if lo == 0 else _dot(w2_s[fs, :], gT[...])
                gate = _dot(w1T[fs, :], hnT[...])
                up = _dot(w3T[fs, :], hnT[...])
                sig = pl.reciprocal(1.0 + jnp.exp2(gate * (-LOG2E)), approx=True)
                silu = gate * sig
                aT[fs, :] = (silu * up).astype(bf16)
                duT[fs, :] = (da * silu).astype(bf16)
                dgT[fs, :] = (da * up * (sig + silu * (1.0 - sig))).astype(bf16)

            def consume(lo, n, first):
                fs = slice(lo, lo + n)
                o_c = _dot(w2T[:, fs], aT[fs, :])
                d_c = _dot(w1_s[:, fs], dgT[fs, :]) + _dot(w3_s[:, fs], duT[fs, :])
                outa[...] += o_c
                if first:
                    dhna[...] = d_c
                else:
                    dhna[...] += d_c

            def accumulate(acc, rows, val):
                if j == 0:
                    acc[rows, :] = val
                else:
                    acc[rows, :] += val

            def weight_grad(which, lo, n):
                fs = slice(lo, lo + n)
                if which == 0:
                    accumulate(dw2a, fs, _dot_nt(aT[fs, :], gT[...]))
                elif which == 1:
                    accumulate(dw1a, fs, _dot_nt(dgT[fs, :], hnT[...]))
                else:
                    accumulate(dw3a, fs, _dot_nt(duT[fs, :], hnT[...]))

            def ln2_bwd(c):
                cs = slice(c * 128, (c + 1) * 128)
                dh = gT[:, cs].astype(f32) + _ln_bwd_fm(dhna[:, cs], hnT[:, cs].astype(f32), r2[:, cs])
                dhT[:, pl.ds(q0 + c * 128, 128)] = dh.astype(bf16)

            for c, (lo, n) in enumerate(fch):
                produce(lo, n)
                if c > 0:
                    consume(*fch[c - 1], c == 1)
                if c > 1:
                    for which in range(3):
                        weight_grad(which, *fch[c - 2])
            consume(*fch[-1], False)
            weight_grad(0, *fch[-2])
            ln2_bwd(0)
            weight_grad(1, *fch[-2])
            ln2_bwd(1)
            weight_grad(2, *fch[-2])
            ln2_bwd(2)
            weight_grad(0, *fch[-1])
            ln2_bwd(3)
            weight_grad(1, *fch[-1])
            obuf[...] = outa[...].astype(bf16).T
            weight_grad(2, *fch[-1])

            dh_b = dhT[:, qs]
            do = _dot(wo_s[...], dh_b)
            li = linv[...]
            hg = H // 4
            for c in range(4):
                rs = slice(c * hg * DH, (c + 1) * hg * DH)
                hs = slice(c * hg, (c + 1) * hg)
                accumulate(dwoa, rs, _dot_nt(oT[rs, :], dh_b))
                do_b = (do[rs].reshape(hg, DH, TQ) * li[hs, None, :]).astype(bf16)
                doT[rs, :] = do_b.reshape(hg * DH, TQ)
                daug[hs, :] = jnp.sum(do_b.astype(f32) * oT32[rs, :].reshape(hg, DH, TQ), axis=1)
            pltpu.make_async_copy(obuf, h2_hbm.at[qs, :], osem.at[0]).start()

            if j == NQ - 1:
                w1T[...] = dw1a[...].astype(bf16)
                w3T[...] = dw3a[...].astype(bf16)
                w2_s[...] = dw2a[...].astype(bf16)
                wo_s[...] = dwoa[...].astype(bf16)
                pltpu.make_async_copy(w1T, dw1T_hbm, sems.at[8]).start()
                pltpu.make_async_copy(w3T, dw3T_hbm, sems.at[9]).start()
                pltpu.make_async_copy(w2_s, dw2_hbm, sems.at[7]).start()
                pltpu.make_async_copy(wo_s, dwo_hbm, sems.at[6]).start()

        with _scope("attn_bwd"):
            attn_step(bprod=(0, pE, 0, dsE))

            def bwd_loop(i, _):
                attn_step(bprod=(2 * i + 1, pO, i, dsO), bcons=(2 * i, pE, i, dsE, q0, None))
                attn_step(bprod=(2 * i + 2, pE, i + 1, dsE), bcons=(2 * i + 1, pO, i, dsO, q0, None))
                return 0

            _loop(last, bwd_loop, 0, BWD_UNROLL)
            attn_step(bprod=(H - 1, pO, last, dsO), bcons=(H - 2, pE, last, dsE, q0, None))
        if j + 1 == NQ:
            parts = []

            def filler(kc):
                if kc % 4 == 0:
                    cs = slice(kc // 4 * 128, (kc // 4 + 1) * 128)
                    parts.append(_dot(wq_s[:, cs], dqT[cs, 0:TX]))

            attn_step(bcons=(H - 1, pO, last, dsO, q0, None), filler=filler)
            return sum(parts[1:], parts[0])
        q_last = qT[head_rows(H - 1), :]
        q_proj(j + 1)
        with _scope("merge"):
            return attn_step(fprod=(0, pE, 0), bcons=(H - 1, pO, last, dsO, q0, q_last))

    q_proj(0)
    l0 = attn_step(fprod=(0, pE, 0))
    for j in range(NQ):
        l0 = tile_body(j, l0)
    dxq0 = l0

    with _scope("epi_dw"):
        dkvT[...] = jnp.concatenate([(dkT[...] * LN2).astype(bf16), dvT[...].astype(bf16)], axis=0)
        dwkvT = _dot_nt(dkvT[...], xnT[...]).astype(bf16)
        dwkvT_s[...] = dwkvT
        dkv_copies = [
            pltpu.make_async_copy(dwkvT_s.at[pl.ds(0, DH), :], dwkT_hbm, sems.at[10]),
            pltpu.make_async_copy(dwkvT_s.at[pl.ds(DH, DH), :], dwvT_hbm, sems.at[11]),
        ]
        for c in dkv_copies:
            c.start()

    def dx_copy(t):
        rows = pl.ds(t * TX, TX)
        return pltpu.make_async_copy(xbuf.at[rows, :], dx_hbm.at[rows, :], xsem.at[t])

    def dx_finish(t, dxn):
        ts = slice(t * TX, (t + 1) * TX)
        dx = dhT[:, ts].astype(f32) + _ln_bwd_fm(dxn, xnT[:, ts].astype(f32), rstd1[0:1, ts])
        xbuf[ts, :] = dx.astype(bf16).T
        dx_copy(t).start()

    with _scope("epi_dx"):
        wkv = wkvT_s[...].T
        prev = None
        for t in range(S // TX):
            ts = slice(t * TX, (t + 1) * TX)
            dxn = (dxq0 if t == 0 else _dot(wq_s[...], dqT[:, ts])) + _dot(wkv, dkvT[:, ts])
            dwq_t = _dot_nt(xnT[:, ts], dqT[:, ts])
            if t == 0:
                dwqa[...] = dwq_t
            else:
                dwqa[...] += dwq_t
            if prev is not None:
                dx_finish(*prev)
            prev = (t, dxn)
    wqT[...] = dwqa[...].astype(bf16)
    dwq_copy = pltpu.make_async_copy(wqT, dwq_hbm, sems.at[5])
    dwq_copy.start()
    dx_finish(*prev)

    pltpu.make_async_copy(obuf, h2_hbm.at[pl.ds(0, TQ), :], osem.at[0]).wait()
    pltpu.make_async_copy(w1T, dw1T_hbm, sems.at[8]).wait()
    pltpu.make_async_copy(w3T, dw3T_hbm, sems.at[9]).wait()
    pltpu.make_async_copy(w2_s, dw2_hbm, sems.at[7]).wait()
    pltpu.make_async_copy(wo_s, dwo_hbm, sems.at[6]).wait()
    dwq_copy.wait()
    for c in dkv_copies:
        c.wait()
    for t in range(S // TX):
        dx_copy(t).wait()


@jax.jit
def pallas_sequential_preLN__grouped_kv_mqa__glu_gated_swiglu__prompt_kernel(
    A_x: jax.Array,
    A_wq: jax.Array,
    A_wk: jax.Array,
    A_wv: jax.Array,
    A_wo: jax.Array,
    B_x: jax.Array,
    B_w1: jax.Array,
    B_w3: jax.Array,
    B_w2: jax.Array,
    grad_out: jax.Array,
):
    del B_x
    V = pltpu.VMEM
    any_spec = pl.BlockSpec(memory_space=pl.ANY)
    scratch = [
        V((D, S), bf16), V((D, S), bf16), V((8, S), f32),
        V((D, D), bf16), V((D, D), bf16), V((D, D), bf16), V((D, D), bf16),
        V((D, F), bf16), V((D, F), bf16), V((F, D), bf16),
        V((F, D), bf16), V((F, D), bf16), V((D, F), bf16),
        V((S, 2 * DH), bf16), V((S, 2 * DH), bf16), V((DH, S), bf16), V((DH, S), bf16),
        V((D, TQ), bf16), V((H, TQ), f32), V((D, TQ), bf16), V((H, TQ), f32),
        V((D, TQ), f32), V((D, TQ), bf16), V((H, TQ), f32),
        V((H // 2, S // 2, TQ), u32), V((H // 2, S // 2, TQ), u32),
        V((S // 2, TQ), u32), V((S // 2, TQ), u32),
        V((D, S), bf16), V((D, S), bf16), V((DH, S), f32), V((DH, S), f32),
        V((2 * DH, S), bf16),
        V((F, D), f32), V((F, D), f32), V((F, D), f32), V((D, D), f32), V((D, D), f32),
        V((F, TQ), bf16), V((F, TQ), bf16), V((F, TQ), bf16),
        V((D, TQ), bf16), V((D, TQ), bf16), V((D, TQ), f32), V((D, TQ), f32),
        V((TQ, D), bf16), V((TQ, D), bf16), V((S, D), bf16),
        V((2 * DH, D), bf16), V((2 * DH, D), bf16),
        pltpu.SemaphoreType.DMA((12,)), pltpu.SemaphoreType.DMA((1,)), pltpu.SemaphoreType.DMA((S // TX,)),
    ]
    sds = jax.ShapeDtypeStruct
    out_shape = (
        sds((S, D), bf16), sds((S, D), bf16),
        sds((D, H * DH), bf16), sds((DH, D), bf16), sds((DH, D), bf16), sds((H * DH, D), bf16),
        sds((F, D), bf16), sds((F, D), bf16), sds((F, D), bf16),
    )
    outs = pl.pallas_call(
        _kernel,
        out_shape=out_shape,
        in_specs=[any_spec, any_spec, any_spec, any_spec, any_spec, any_spec, any_spec, any_spec, any_spec],
        out_specs=(any_spec, any_spec, any_spec, any_spec, any_spec, any_spec, any_spec, any_spec, any_spec),
        scratch_shapes=scratch,
        compiler_params=pltpu.CompilerParams(vmem_limit_bytes=127 * 1024 * 1024),
        name="preln_mqa_swiglu_fwdbwd",
    )(A_x.reshape(S, D), A_wq, A_wk.T, A_wv.T, A_wo, B_w1.T, B_w3.T, B_w2, grad_out.reshape(S, D))
    h2, dx, dwq, dwkT, dwvT, dwo, dw1T, dw3T, dw2 = outs
    return (h2.reshape(1, S, D), dx.reshape(1, S, D), dwq, dwkT.T, dwvT.T, dwo, dw1T.T, dw3T.T, dw2)
```
